```python
import os as _os
_os.environ.setdefault("JAX_PLATFORMS", "cpu")
import jax
import jax.numpy as jnp

def _softmax(x, axis=-1):
    return jax.nn.softmax(x, axis=axis)
def _gelu(x):
    return jax.nn.gelu(x, approximate=True)
def _silu(x):
    return jax.nn.silu(x)
def _sigmoid(x):
    return jax.nn.sigmoid(x)
def _layernorm(x, axis=-1, eps=1e-5):
    m = jnp.mean(x, axis=axis, keepdims=True)
    v = jnp.var(x, axis=axis, keepdims=True)
    return (x - m) / jnp.sqrt(v + eps)
def _scatter_add(tgt, idx, src, axis=0):
    return tgt.at[idx].add(src)
def _segment_sum(src, seg, n):
    return jax.ops.segment_sum(src, seg, n)
class _Rng:
    def __init__(self, key):
        self._k = key
    def _next(self):
        self._k, sub = jax.random.split(self._k)
        return sub
    def normal(self, shape):
        return jax.random.normal(self._next(), shape, dtype=jnp.bfloat16)
    def randint(self, lo, hi, shape):
        return jax.random.randint(self._next(), shape, lo, hi, dtype=jnp.int32)
    def uniform(self, shape, lo=0.0, hi=1.0):
        return jax.random.uniform(self._next(), shape, jnp.bfloat16, lo, hi)
    def permutation(self, n):
        return jax.random.permutation(self._next(), n)


kernel_name = 'interleave_layers__linear_kernel_hedgehog__ssm_conv_s4__prompt'

def setup_inputs():
    _rng = _Rng(jax.random.key(int.from_bytes(__import__("os").urandom(4), "little")))
    _w = (lambda a: (lambda t: t.astype(jnp.bfloat16) if jnp.issubdtype(t.dtype, jnp.floating) else t)(jnp.asarray(a)))
    def _A_setup():
        B, S, D, H = 1, 2048, 512, 32
        Dh = D // H
        return {
            "x": _w((lambda *s: _rng.normal(s) * 0.05)(B, S, D)),
            "wqkv": _w((lambda *s: _rng.normal(s) * 0.4)(D, 3 * D)),
            "w_phi": _w((lambda *s: _rng.normal(s) * 0.4)(H, Dh, Dh) * (Dh ** -0.5)),
            "wo": _w((lambda *s: _rng.normal(s) * 0.05)(D, D)),
        }
    _A_in = _A_setup()

    def _B_setup():
        B, L, D, N = 1, 2048, 512, 128
        A_re = -jnp.exp((lambda *s: _rng.normal(s) * 0.2)(D, N))
        A_im = jnp.pi * (lambda *s: _rng.normal(s) * 0.2)(D, N)
        B_re = (lambda *s: _rng.normal(s) * 0.2)(D, N)
        B_im = (lambda *s: _rng.normal(s) * 0.2)(D, N)
        C_re = (lambda *s: _rng.normal(s) * 0.2)(D, N)
        C_im = (lambda *s: _rng.normal(s) * 0.2)(D, N)
        log_dt = (lambda *s: _rng.normal(s) * 0.2)(D) * 0.5 - 4.0
        Dskip = (lambda *s: _rng.normal(s) * 0.2)(D)
        return {
            "u": _w((lambda *s: _rng.normal(s) * 0.05)(B, L, D)),
            "A_re": _w(A_re),
            "A_im": _w(A_im),
            "B_re": _w(B_re),
            "B_im": _w(B_im),
            "C_re": _w(C_re),
            "C_im": _w(C_im),
            "log_dt": _w(log_dt),
            "Dskip": _w(Dskip),
        }
    _B_in = _B_setup()

    return {
        "A_x": _A_in["x"],
        "A_wqkv": _A_in["wqkv"],
        "A_w_phi": _A_in["w_phi"],
        "A_wo": _A_in["wo"],
        "B_u": _B_in["u"],
        "B_A_re": _B_in["A_re"],
        "B_A_im": _B_in["A_im"],
        "B_B_re": _B_in["B_re"],
        "B_B_im": _B_in["B_im"],
        "B_C_re": _B_in["C_re"],
        "B_C_im": _B_in["C_im"],
        "B_log_dt": _B_in["log_dt"],
        "B_Dskip": _B_in["Dskip"],
    }

def reference(A_x, A_wqkv, A_w_phi, A_wo, B_u, B_A_re, B_A_im, B_B_re, B_B_im, B_C_re, B_C_im, B_log_dt, B_Dskip):
    def _A_ref(x, wqkv, w_phi, wo):
        B, S, D = x.shape
        H = 32; Dh = D // H
        qkv = (lambda x, *d: x.transpose(*d))((x @ wqkv).reshape(B, S, 3, H, Dh), 2, 0, 3, 1, 4)
        q, k, v = qkv[0], qkv[1], qkv[2]
        pq = jnp.einsum("bhsd,hdf->bhsf", q, w_phi)
        pk = jnp.einsum("bhsd,hdf->bhsf", k, w_phi)
        phi_q = jnp.concatenate([_softmax(pq, axis=-1), _softmax(-pq, axis=-1)], axis=-1)
        phi_k = jnp.concatenate([_softmax(pk, axis=-1), _softmax(-pk, axis=-1)], axis=-1)
        kv = jnp.einsum("bhsf,bhsd->bhfd", phi_k, v)
        z  = jnp.einsum("bhsf->bhf", phi_k)
        num = jnp.einsum("bhqf,bhfd->bhqd", phi_q, kv)
        den = jnp.einsum("bhqf,bhf->bhq", phi_q, z)[..., None] + 1e-6
        o = num / den
        return (lambda x, *d: x.transpose(*d))(o, 0, 2, 1, 3).reshape(B, S, D) @ wo

    def _B_ref(u, A_re, A_im, B_re, B_im, C_re, C_im, log_dt, Dskip):
        Bsz, L, D = u.shape
        dt = jnp.exp(log_dt)[:, None]
        A = A_re + 1j * A_im
        Bc = B_re + 1j * B_im
        Cc = C_re + 1j * C_im
        logdA = dt * A
        dB = dt * Bc
        l = (lambda x, dt: x.astype(dt))(jnp.arange(L), A_re.dtype)
        P = jnp.exp(logdA[:, :, None] * l[None, None, :])
        K = jnp.einsum("dn,dnl,dn->dl", Cc, P, dB).real
        L2 = 2 * L
        Kp = jnp.pad(K, ((0, 0), (0, L)))
        up = (lambda x, *d: x.transpose(*d))(u, 0, 2, 1)
        up = jnp.pad(up, ((0, 0), (0, 0), (0, L)))
        Kf = (lambda x, axes=(-2,-1): jnp.fft.rfft2(x.astype(jnp.float32), axes=axes))(Kp[:, None, :], axes=(-2, -1))
        Uf = (lambda x, axes=(-2,-1): jnp.fft.rfft2(x.astype(jnp.float32), axes=axes))(up[:, :, None, :], axes=(-2, -1))
        Yf = Uf * Kf[None, :, :, :]
        y = (lambda x, s, axes=(-2,-1): jnp.fft.irfft2(x, s=s, axes=axes).astype(jnp.bfloat16))(Yf, (1, L2), axes=(-2, -1))[:, :, 0, :L]
        y = (lambda x, *d: x.transpose(*d))(y, 0, 2, 1) + u * Dskip[None, None, :]
        return y

    x = A_x
    x = x + _A_ref(_layernorm(x, axis=-1), A_wqkv, A_w_phi, A_wo)
    x = x + _B_ref(_layernorm(x, axis=-1), B_A_re, B_A_im, B_B_re, B_B_im, B_C_re, B_C_im, B_log_dt, B_Dskip)
    x = x + _A_ref(_layernorm(x, axis=-1), A_wqkv, A_w_phi, A_wo)
    x = x + _B_ref(_layernorm(x, axis=-1), B_A_re, B_A_im, B_B_re, B_B_im, B_C_re, B_C_im, B_log_dt, B_Dskip)
    return x
```

```python
import os
import numpy as np
import jax
import jax.numpy as jnp
from jax import lax
import jax.experimental.pallas as pl
import jax.experimental.pallas.tpu as pltpu

S = 2048
D = 512
NT = 16
PS = 513
NFFT = 4096
BF = jnp.bfloat16
F32 = jnp.float32


def _dft_constants():
    n1 = np.arange(16)[None, :]
    k1 = np.arange(17)[:, None]
    ang = -2.0 * np.pi * (n1 * k1) / 32.0
    f1 = np.concatenate([np.cos(ang), np.sin(ang)[1:16]], axis=0)
    eye8 = np.eye(8)
    s1 = np.kron(f1, eye8)
    s1k = np.einsum("pn,ab->panb", f1, eye8)
    s1k = np.transpose(s1k, (0, 1, 3, 2)).reshape(256, 128)
    n1c = np.arange(16)[:, None]
    k1r = np.arange(17)[None, :]
    ang2 = 2.0 * np.pi * (n1c * k1r) / 32.0
    wre = 2.0 * np.cos(ang2)
    wre[:, 0] = 1.0
    wre[:, 16] = np.cos(np.pi * np.arange(16))
    wim = -2.0 * np.sin(ang2)[:, 1:16]
    g4 = np.concatenate([wre, wim], axis=1)
    s4 = np.kron(g4, eye8)
    n2 = np.arange(128)[:, None]
    k2 = np.arange(128)[None, :]
    f2 = np.zeros((17, 3, 128, 128), np.float64)
    for k in range(17):
        a = -2.0 * np.pi * ((n2 * (k + 32 * k2)) % NFFT) / NFFT
        fr, fi = np.cos(a), np.sin(a)
        f2[k, 0] = fr
        if k in (0, 16):
            f2[k, 1] = fi
            f2[k, 2] = fi
        else:
            f2[k, 1] = fr + fi
            f2[k, 2] = fi - fr
    import ml_dtypes
    bf = ml_dtypes.bfloat16
    return (s1.astype(np.float32).astype(bf), s1k.astype(np.float32).astype(bf),
            s4.astype(np.float32).astype(bf), f2.astype(np.float32).astype(bf))


_S1, _S1K, _S4, _F2 = _dft_constants()

_NN = (((1,), (0,)), ((), ()))
_NTD = (((1,), (1,)), ((), ()))


def _mm(a, b, dn=_NN):
    return lax.dot_general(a, b, dn, preferred_element_type=F32)


def _cmul(ar, ai, br, bi):
    return ar * br - ai * bi, ar * bi + ai * br


def _sincos(x):
    kq = jnp.round(x * 0.6366197723675814)
    r = x - kq * 1.5703125
    r = r - kq * 4.837512969970703e-4
    r = r - kq * 7.549790126404332e-8
    r2 = r * r
    sn = r + r * r2 * (-1.6666654611e-1 + r2 * (8.3321608736e-3 + r2 * -1.9515295891e-4))
    cs = 1.0 + r2 * (-0.5 + r2 * (4.166664568298827e-2 + r2 * (-1.388731625493765e-3 + r2 * 2.443315711809948e-5)))
    ki = kq.astype(jnp.int32)
    swap = (ki & 1) == 1
    s_ = jnp.where(swap, cs, sn)
    c_ = jnp.where(swap, sn, cs)
    s_ = jnp.where((ki & 2) == 2, -s_, s_)
    c_ = jnp.where(((ki + 1) & 2) == 2, -c_, c_)
    return s_, c_


def _layernorm_cols(x):
    m = jnp.mean(x, axis=0, keepdims=True)
    xc = x - m
    v = jnp.mean(xc * xc, axis=0, keepdims=True)
    return xc * lax.rsqrt(v + 1e-5)


def _dual_softmax(p):
    if False and p.shape[1] > 128:
        return jnp.concatenate([_dual_softmax(p[:, t:t + 128]) for t in range(0, p.shape[1], 128)], axis=1)
    c = p.shape[1]
    p3 = p.reshape(16, 8, c)
    mx = jnp.max(p3, axis=0, keepdims=True)
    mn = jnp.min(p3, axis=0, keepdims=True)
    ep = jnp.exp(p3 - mx)
    en = jnp.exp(mn - p3)
    rp = 1.0 / jnp.sum(ep, axis=0, keepdims=True)
    rn = 1.0 / jnp.sum(en, axis=0, keepdims=True)
    return jnp.concatenate([(ep * rp).reshape(128, c), (en * rn).reshape(128, c)], axis=0)


def _kernel(x_hbm, wqkv_hbm, wphi_ref, wo_hbm, are_ref, aim_ref, bre_ref, bim_ref,
            cre_ref, cim_ref, ldt_ref, dsk_ref, s1_ref, s1k_ref, s4_ref, f2_hbm,
            o_hbm,
            x_ref, wqkv_ref, wo_ref, f2_ref, o_ref, kt_s, sems, osems,
            xT, uT, xn_s, pln, kf, wT, woT, kvacc, zacc, kvT, zbr, zbi, war, wai, dskb, z8r_s, z8i_s, zkr_s, zki_s, z64r_s, z64i_s):
    SU = int(os.environ.get('SU', 32))
    AU = 1
    TU = int(os.environ.get('TU', 5))
    CT = 8
    C = 128 * CT

    cp_f2 = pltpu.make_async_copy(f2_hbm, f2_ref, sems.at[0])
    cp_w = pltpu.make_async_copy(wqkv_hbm, wqkv_ref, sems.at[1])
    cp_wo = pltpu.make_async_copy(wo_hbm, wo_ref, sems.at[2])
    cp_x = pltpu.make_async_copy(x_hbm, x_ref, sems.at[3])
    cp_x.start()
    cp_f2.start()
    cp_w.start()
    cp_wo.start()

    def iota(shape, dim):
        return lax.broadcasted_iota(jnp.int32, shape, dim)

    ldt = jnp.broadcast_to(ldt_ref[...].astype(F32).reshape(1, D), (128, D)).T
    dt = jnp.exp(ldt).astype(BF).astype(F32)
    dskb[...] = jnp.broadcast_to(dsk_ref[...].astype(F32).reshape(1, D), (128, D)).T

    def fft_stage2_fwd(k, first):
        ar = pln[k]
        if first:
            arb = ar.astype(BF)
            return _mm(arb, f2_ref[k, 0]), _mm(arb, f2_ref[k, 1])
        ai = pln[16 + k]
        p1 = _mm((ar + ai).astype(BF), f2_ref[k, 0])
        p2 = _mm(ai.astype(BF), f2_ref[k, 1])
        p3 = _mm(ar.astype(BF), f2_ref[k, 2])
        return p1 - p2, p1 + p3

    lam_r = dt * are_ref[...].astype(F32)
    lam_i = dt * aim_ref[...].astype(F32)
    mag = jnp.exp(lam_r)
    sn_, cs_ = _sincos(lam_i)
    z1r = mag * cs_
    z1i = mag * sn_
    dbr = dt * bre_ref[...].astype(F32)
    dbi = dt * bim_ref[...].astype(F32)
    wr, wi = _cmul(cre_ref[...].astype(F32), cim_ref[...].astype(F32), dbr, dbi)
    pr = jnp.ones_like(z1r)
    pi = jnp.zeros_like(z1r)
    for s in range(8):
        zbr[s * PS:s * PS + D, :] = pr
        zbi[s * PS:s * PS + D, :] = pi
        pr, pi = _cmul(pr, pi, z1r, z1i)
    z8r_s[...] = pr
    z8i_s[...] = pi
    for _ in range(3):
        pr, pi = pr * pr - pi * pi, 2.0 * pr * pi
    z64r_s[...] = pr
    z64i_s[...] = pi
    pr, pi = pr * pr - pi * pi, 2.0 * pr * pi
    qr, qi = wr, wi
    for a in range(8):
        war[a * PS:a * PS + D, :] = qr
        wai[a * PS:a * PS + D, :] = -qi
        qr, qi = _cmul(qr, qi, pr, pi)
    for _ in range(3):
        pr, pi = pr * pr - pi * pi, 2.0 * pr * pi
    zkr_s[...] = pr
    zki_s[...] = pi

    KU = int(os.environ.get('KU', 4))

    cp_x.wait()

    def kgen(gg, _):
        blk = x_ref[pl.ds(pl.multiple_of(gg * 128, 128), 128), :].T.astype(F32)
        xT[gg] = blk
        lo = lax.broadcasted_iota(jnp.int32, (16, 128), 1) < 64

        def row(ref, d):
            return jnp.broadcast_to(ref[pl.ds(d, 1), :], (8, 128))

        for q in range(KU):
            g = gg * KU + q
            outs = []
            for j in range(4):
                lr, li, tr, ti = [], [], [], []
                for d in (g * 8 + 2 * j, g * 8 + 2 * j + 1):
                    a0r = war[pl.ds(d, 8, stride=PS), :]
                    a0i = wai[pl.ds(d, 8, stride=PS), :]
                    zkr, zki = row(zkr_s, d), row(zki_s, d)
                    zhr, zhi = row(z64r_s, d), row(z64i_s, d)
                    a1r = a0r * zkr + a0i * zki
                    a1i = a0i * zkr - a0r * zki
                    lr += [a0r, a1r, a0r * zhr + a0i * zhi, a1r * zhr + a1i * zhi]
                    li += [a0i, a1i, a0i * zhr - a0r * zhi, a1i * zhr - a1r * zhi]
                    er = zbr[pl.ds(d, 8, stride=PS), :]
                    ei = zbi[pl.ds(d, 8, stride=PS), :]
                    z8r, z8i = row(z8r_s, d), row(z8i_s, d)
                    tr.append(er)
                    ti.append(ei)
                    for i in range(7):
                        er, ei = _cmul(er, ei, z8r, z8i)
                        tr.append(er)
                        ti.append(ei)
                lhs = jnp.concatenate([jnp.concatenate(lr, axis=0),
                                       jnp.concatenate(li, axis=0)], axis=1).astype(BF)
                rhs = jnp.concatenate([jnp.concatenate(tr, axis=0),
                                       jnp.concatenate(ti, axis=0)], axis=1).astype(BF)
                o = _mm(lhs, rhs, _NTD)
                ev = jnp.where(lo, o[0:16], o[32:48])
                od = jnp.where(lo, o[16:32], o[48:64])
                outs.append(jnp.where(lo, ev, pltpu.roll(od, 64, 1)))
                outs.append(jnp.where(lo, pltpu.roll(ev, 64, 1), od))
            kt_s[g] = jnp.concatenate(outs, axis=0).astype(BF)
        return _
    lax.fori_loop(0, D // 8 // KU, kgen, None)

    def st1k(gg, _):
        tiles = [kt_s[gg * SU + j] for j in range(SU)]
        res = _mm(s1k_ref[...], jnp.concatenate(tiles, axis=1))
        for j in range(SU):
            sl = pl.ds(pl.multiple_of((gg * SU + j) * 8, 8), 8)
            pln[:, sl, :] = res[:, 128 * j:128 * (j + 1)].reshape(32, 8, 128)
        return _
    lax.fori_loop(0, D // 8 // SU, st1k, None)
    cp_f2.wait()

    inv_n = 1.0 / NFFT
    for k in (0, 16):
        fr_, fi_ = fft_stage2_fwd(k, True)
        kf[k, 0] = fr_ * inv_n
        kf[k, 1] = fi_ * inv_n

    def kf_loop(kk, _):
        for u in range(TU):
            k = 1 + kk * TU + u
            fr_, fi_ = fft_stage2_fwd(k, False)
            kf[k, 0] = fr_ * inv_n
            kf[k, 1] = fi_ * inv_n
        return _
    lax.fori_loop(0, 15 // TU, kf_loop, None)

    cp_w.wait()
    cp_wo.wait()
    r = iota((128, 128), 0)
    c = iota((128, 128), 1)
    bmask = (r % 8) == (c // 16)
    pmat = ((r // 8 == c % 16) & (r % 8 == c // 16)).astype(BF)
    wp2 = wphi_ref[...].reshape(256, 32)
    rx = (iota((128, 256), 0) // 8 == iota((128, 256), 1) % 16).astype(BF)
    sel = (iota((32, D), 0) == iota((32, D), 1) // 16).astype(BF)
    uall = _mm(wp2, sel)
    vall = jnp.where(iota((256, D), 0) // 16 == iota((256, D), 1) % 16, uall, 0.0).astype(BF)
    bdT = _mm(rx, vall)
    for g in range(4):
        bg = jnp.where(bmask, bdT[:, 128 * g:128 * (g + 1)], 0.0).astype(BF)
        wT[128 * g:128 * (g + 1), :] = _mm(bg, wqkv_ref[:, 128 * g:128 * (g + 1)], _NTD).astype(BF)
        wT[512 + 128 * g:512 + 128 * (g + 1), :] = _mm(
            bg, wqkv_ref[:, 512 + 128 * g:512 + 128 * (g + 1)], _NTD).astype(BF)
        wT[1024 + 128 * g:1024 + 128 * (g + 1), :] = _mm(
            pmat, wqkv_ref[:, 1024 + 128 * g:1024 + 128 * (g + 1)], _NTD).astype(BF)
        wog = _mm(pmat, wo_ref[128 * g:128 * (g + 1), :])
        woT[:, 128 * g:128 * (g + 1)] = wog.T.astype(BF)

    def load_chunk(ref, i):
        return jnp.concatenate([ref[i * CT + t] for t in range(CT)], axis=1)

    def store_chunk(ref, i, val):
        for t in range(CT):
            ref[i * CT + t] = val[:, 128 * t:128 * (t + 1)]

    def layer(_l, _c):
        kvacc[...] = jnp.zeros(kvacc.shape, F32)
        zacc[...] = jnp.zeros(zacc.shape, F32)

        def ln_chunk(i):
            store_chunk(xn_s, i, _layernorm_cols(load_chunk(xT, i)).astype(BF))

        if '0' != '0':
            for u in range(AU):
                ln_chunk(u)
        NI = NT // CT // AU

        def pass1(ii, _):
            if '0' == '2':
                for u in range(AU):
                    ln_chunk(jnp.minimum(ii + 1, NI - 1) * AU + u)
            for u in range(AU):
                i = ii * AU + u
                if '0' == '0':
                    ln_chunk(i)
                xn = load_chunk(xn_s, i)
                kvp = _mm(wT[512:1536, :], xn)
                for g in range(4):
                    phi = _dual_softmax(kvp[128 * g:128 * (g + 1)])
                    vg = kvp[512 + 128 * g:512 + 128 * (g + 1)].astype(BF)
                    kvacc[g] += _mm(phi.astype(BF), vg, _NTD)
                    zs = phi[:, 0:128]
                    for t in range(1, CT):
                        zs = zs + phi[:, 128 * t:128 * (t + 1)]
                    zacc[g] += zs
            if '0' == '1':
                for u in range(AU):
                    ln_chunk(jnp.minimum(ii + 1, NI - 1) * AU + u)
            return _
        lax.fori_loop(0, NT // CT // AU, pass1, None)

        hm = (iota((144, 256), 0) % 8) == (iota((144, 256), 1) % 8)
        for g in range(4):
            zcol = jnp.sum(zacc[g], axis=1, keepdims=True)
            ext = jnp.concatenate([kvacc[g], jnp.broadcast_to(zcol, (256, 128))], axis=1)
            extT = ext.T
            kvT[g] = jnp.where(hm, extT[0:144], 0.0).astype(BF)

        def lnu_chunk(i):
            store_chunk(uT, i, _layernorm_cols(load_chunk(xT, i)))

        def pass2(ii, _):
            if '0' == '1':
                for u in range(AU):
                    lnu_chunk(jnp.maximum(ii - 1, 0) * AU + u)
            for u in range(AU):
                i = ii * AU + u
                xn = load_chunk(xn_s, i)
                pq = _mm(wT[0:512, :], xn)
                os_ = []
                for g in range(4):
                    phi = _dual_softmax(pq[128 * g:128 * (g + 1)]).astype(BF)
                    nd = _mm(kvT[g], phi)
                    rden = 1.0 / (nd[128:136] + 1e-6)
                    os_.append((nd[0:128].reshape(16, 8, C) * rden[None]).reshape(128, C))
                o = jnp.concatenate(os_, axis=0).astype(BF)
                xnew = load_chunk(xT, i) + _mm(woT[...], o)
                store_chunk(xT, i, xnew)
                if '0' == '0':
                    store_chunk(uT, i, _layernorm_cols(xnew))
            return _
        lax.fori_loop(0, NT // CT // AU, pass2, None)
        if '0' == '1':
            for u in range(AU):
                lnu_chunk((NI - 1) * AU + u)

        def st1(gg, _):
            tiles = []
            for j in range(SU):
                sl = pl.ds(pl.multiple_of((gg * SU + j) * 8, 8), 8)
                tiles.append(uT[:, sl, :].reshape(128, 128).astype(BF))
            res = _mm(s1_ref[...], jnp.concatenate(tiles, axis=1))
            for j in range(SU):
                sl = pl.ds(pl.multiple_of((gg * SU + j) * 8, 8), 8)
                pln[:, sl, :] = res[:, 128 * j:128 * (j + 1)].reshape(32, 8, 128)
            return _
        lax.fori_loop(0, D // 8 // SU, st1, None)

        for k in (0, 16):
            ur, ui = fft_stage2_fwd(k, True)
            yr, yi = _cmul(ur, ui, kf[k, 0], kf[k, 1])
            pln[k] = (_mm(yr.astype(BF), f2_ref[k, 0], _NTD)
                      + _mm(yi.astype(BF), f2_ref[k, 1], _NTD))

        def st23(kk, _):
            for u in range(TU):
                k = 1 + kk * TU + u
                ur, ui = fft_stage2_fwd(k, False)
                yr, yi = _cmul(ur, ui, kf[k, 0], kf[k, 1])
                q1 = _mm((yr + yi).astype(BF), f2_ref[k, 0], _NTD)
                q2 = _mm(yr.astype(BF), f2_ref[k, 1], _NTD)
                q3 = _mm(yi.astype(BF), f2_ref[k, 2], _NTD)
                pln[k] = q1 + q3
                pln[16 + k] = q1 - q2
            return _
        lax.fori_loop(0, 15 // TU, st23, None)

        def st4(gg, _):
            tiles = []
            for j in range(SU):
                sl = pl.ds(pl.multiple_of((gg * SU + j) * 8, 8), 8)
                tiles.append(pln[:, sl, :].reshape(256, 128).astype(BF))
            res = _mm(s4_ref[...], jnp.concatenate(tiles, axis=1))
            for j in range(SU):
                sl = pl.ds(pl.multiple_of((gg * SU + j) * 8, 8), 8)
                y = res[:, 128 * j:128 * (j + 1)].reshape(16, 8, 128)
                xT[:, sl, :] = xT[:, sl, :] + y + uT[:, sl, :] * dskb[sl, :][None]
            return _
        lax.fori_loop(0, D // 8 // SU, st4, None)
        return _c

    lax.fori_loop(0, 2, layer, None)

    ocps = []
    for ch in range(4):
        for j in range(4):
            i = ch * 4 + j
            o_ref[i * 128:(i + 1) * 128, :] = xT[i].astype(o_ref.dtype).T
        cp = pltpu.make_async_copy(o_ref.at[pl.ds(ch * 512, 512), :], o_hbm.at[pl.ds(ch * 512, 512), :],
                                   osems.at[ch])
        cp.start()
        ocps.append(cp)
    for cp in ocps:
        cp.wait()


def _build(interpret=False):
    def run(A_x, A_wqkv, A_w_phi, A_wo, B_u, B_A_re, B_A_im, B_B_re, B_B_im, B_C_re, B_C_im,
            B_log_dt, B_Dskip):
        del B_u
        x2 = A_x.reshape(S, D)
        wphi, ldt, dsk = jnp.transpose(A_w_phi, (1, 2, 0)), B_log_dt, B_Dskip
        scratch = [
            pltpu.VMEM((S, D), BF),
            pltpu.VMEM((D, 3 * D), BF),
            pltpu.VMEM((D, D), BF),
            pltpu.VMEM((17, 3, 128, 128), BF),
            pltpu.VMEM((S, D), A_x.dtype),
            pltpu.VMEM((64, 128, 128), BF),
            pltpu.SemaphoreType.DMA((4,)),
            pltpu.SemaphoreType.DMA((4,)),
            pltpu.VMEM((NT, D, 128), F32),
            pltpu.VMEM((NT, D, 128), F32),
            pltpu.VMEM((NT, D, 128), BF),
            pltpu.VMEM((32, D, 128), F32),
            pltpu.VMEM((17, 2, D, 128), F32),
            pltpu.VMEM((3 * D, D), BF),
            pltpu.VMEM((D, D), BF),
            pltpu.VMEM((4, 256, 128), F32),
            pltpu.VMEM((4, 256, 128), F32),
            pltpu.VMEM((4, 144, 256), BF),
            pltpu.VMEM((8 * PS, 128), F32),
            pltpu.VMEM((8 * PS, 128), F32),
            pltpu.VMEM((8 * PS, 128), F32),
            pltpu.VMEM((8 * PS, 128), F32),
            pltpu.VMEM((D, 128), F32),
            pltpu.VMEM((D, 128), F32),
            pltpu.VMEM((D, 128), F32),
            pltpu.VMEM((D, 128), F32),
            pltpu.VMEM((D, 128), F32),
            pltpu.VMEM((D, 128), F32),
            pltpu.VMEM((D, 128), F32),
        ]
        any_ = pl.BlockSpec(memory_space=pl.ANY)
        vm = pl.BlockSpec(memory_space=pltpu.VMEM)
        out = pl.pallas_call(
            _kernel,
            out_shape=jax.ShapeDtypeStruct((S, D), A_x.dtype),
            scratch_shapes=scratch,
            in_specs=[any_, any_, vm, any_] + [vm] * 11 + [any_],
            out_specs=any_,
            compiler_params=pltpu.CompilerParams(vmem_limit_bytes=100 * 1024 * 1024),
            interpret=interpret,
        )(x2, A_wqkv, wphi, A_wo, B_A_re, B_A_im, B_B_re, B_B_im, B_C_re, B_C_im, ldt, dsk,
          _S1, _S1K, _S4, _F2)
        return out.reshape(A_x.shape)
    return run


pallas_interleave_layers__linear_kernel_hedgehog__ssm_conv_s4__prompt_kernel = jax.jit(_build(False))
```

```python
import numpy as np
import jax
import jax.numpy as jnp
from jax import lax
import jax.experimental.pallas as pl
import jax.experimental.pallas.tpu as pltpu

S = 2048
D = 512
NT = 16
PS = 513
NFFT = 4096
BF = jnp.bfloat16
F32 = jnp.float32


def _dft_constants():
    n1 = np.arange(16)[None, :]
    k1 = np.arange(17)[:, None]
    ang = -2.0 * np.pi * (n1 * k1) / 32.0
    f1 = np.concatenate([np.cos(ang), np.sin(ang)[1:16]], axis=0)
    eye8 = np.eye(8)
    s1 = np.kron(f1, eye8)
    s1k = np.einsum("pn,ab->panb", f1, eye8)
    s1k = np.transpose(s1k, (0, 1, 3, 2)).reshape(256, 128)
    n1c = np.arange(16)[:, None]
    k1r = np.arange(17)[None, :]
    ang2 = 2.0 * np.pi * (n1c * k1r) / 32.0
    wre = 2.0 * np.cos(ang2)
    wre[:, 0] = 1.0
    wre[:, 16] = np.cos(np.pi * np.arange(16))
    wim = -2.0 * np.sin(ang2)[:, 1:16]
    g4 = np.concatenate([wre, wim], axis=1)
    s4 = np.kron(g4, eye8)
    n2 = np.arange(128)[:, None]
    k2 = np.arange(128)[None, :]
    f2 = np.zeros((17, 3, 128, 128), np.float64)
    for k in range(17):
        a = -2.0 * np.pi * ((n2 * (k + 32 * k2)) % NFFT) / NFFT
        fr, fi = np.cos(a), np.sin(a)
        f2[k, 0] = fr
        if k in (0, 16):
            f2[k, 1] = fi
            f2[k, 2] = fi
        else:
            f2[k, 1] = fr + fi
            f2[k, 2] = fi - fr
    import ml_dtypes
    bf = ml_dtypes.bfloat16
    return (s1.astype(np.float32).astype(bf), s1k.astype(np.float32).astype(bf),
            s4.astype(np.float32).astype(bf), f2.astype(np.float32).astype(bf))


_S1, _S1K, _S4, _F2 = _dft_constants()

_NN = (((1,), (0,)), ((), ()))
_NTD = (((1,), (1,)), ((), ()))


def _mm(a, b, dn=_NN):
    return lax.dot_general(a, b, dn, preferred_element_type=F32)


def _cmul(ar, ai, br, bi):
    return ar * br - ai * bi, ar * bi + ai * br


def _sincos(x):
    kq = jnp.round(x * 0.6366197723675814)
    r = x - kq * 1.5703125
    r = r - kq * 4.837512969970703e-4
    r = r - kq * 7.549790126404332e-8
    r2 = r * r
    sn = r + r * r2 * (-1.6666654611e-1 + r2 * (8.3321608736e-3 + r2 * -1.9515295891e-4))
    cs = 1.0 + r2 * (-0.5 + r2 * (4.166664568298827e-2 + r2 * (-1.388731625493765e-3 + r2 * 2.443315711809948e-5)))
    ki = kq.astype(jnp.int32)
    swap = (ki & 1) == 1
    s_ = jnp.where(swap, cs, sn)
    c_ = jnp.where(swap, sn, cs)
    s_ = jnp.where((ki & 2) == 2, -s_, s_)
    c_ = jnp.where(((ki + 1) & 2) == 2, -c_, c_)
    return s_, c_


def _layernorm_cols(x):
    m = jnp.mean(x, axis=0, keepdims=True)
    xc = x - m
    v = jnp.mean(xc * xc, axis=0, keepdims=True)
    return xc * lax.rsqrt(v + 1e-5)


def _dual_softmax(p):
    c = p.shape[1]
    p3 = p.reshape(16, 8, c)
    mx = jnp.max(p3, axis=0, keepdims=True)
    mn = jnp.min(p3, axis=0, keepdims=True)
    ep = jnp.exp(p3 - mx)
    en = jnp.exp(mn - p3)
    rp = 1.0 / jnp.sum(ep, axis=0, keepdims=True)
    rn = 1.0 / jnp.sum(en, axis=0, keepdims=True)
    return jnp.concatenate([(ep * rp).reshape(128, c), (en * rn).reshape(128, c)], axis=0)


def _kernel(x_hbm, wqkv_hbm, wphi_ref, wo_hbm, are_ref, aim_ref, bre_ref, bim_ref,
            cre_ref, cim_ref, ldt_ref, dsk_ref, s1_ref, s1k_ref, s4_ref, f2_hbm,
            o_hbm,
            x_ref, wqkv_ref, wo_ref, f2_ref, o_ref, kt_s, sems, osems,
            xT, uT, xn_s, pln, kf, wT, woT, kvacc, zacc, kvT, zbr, zbi, war, wai, dskb, z8r_s, z8i_s, zkr_s, zki_s, z64r_s, z64i_s):
    SU = 32
    AU = 1
    TU = 5
    CT = 8
    C = 128 * CT

    cp_f2 = pltpu.make_async_copy(f2_hbm, f2_ref, sems.at[0])
    cp_w = pltpu.make_async_copy(wqkv_hbm, wqkv_ref, sems.at[1])
    cp_wo = pltpu.make_async_copy(wo_hbm, wo_ref, sems.at[2])
    cp_x = pltpu.make_async_copy(x_hbm, x_ref, sems.at[3])
    cp_x.start()
    cp_f2.start()
    cp_w.start()
    cp_wo.start()

    def iota(shape, dim):
        return lax.broadcasted_iota(jnp.int32, shape, dim)

    ldt = jnp.broadcast_to(ldt_ref[...].astype(F32).reshape(1, D), (128, D)).T
    dt = jnp.exp(ldt).astype(BF).astype(F32)
    dskb[...] = jnp.broadcast_to(dsk_ref[...].astype(F32).reshape(1, D), (128, D)).T

    def fft_stage2_fwd(k, first):
        ar = pln[k]
        if first:
            arb = ar.astype(BF)
            return _mm(arb, f2_ref[k, 0]), _mm(arb, f2_ref[k, 1])
        ai = pln[16 + k]
        p1 = _mm((ar + ai).astype(BF), f2_ref[k, 0])
        p2 = _mm(ai.astype(BF), f2_ref[k, 1])
        p3 = _mm(ar.astype(BF), f2_ref[k, 2])
        return p1 - p2, p1 + p3

    lam_r = dt * are_ref[...].astype(F32)
    lam_i = dt * aim_ref[...].astype(F32)
    mag = jnp.exp(lam_r)
    sn_, cs_ = _sincos(lam_i)
    z1r = mag * cs_
    z1i = mag * sn_
    dbr = dt * bre_ref[...].astype(F32)
    dbi = dt * bim_ref[...].astype(F32)
    wr, wi = _cmul(cre_ref[...].astype(F32), cim_ref[...].astype(F32), dbr, dbi)
    pr = jnp.ones_like(z1r)
    pi = jnp.zeros_like(z1r)
    for s in range(8):
        zbr[s * PS:s * PS + D, :] = pr
        zbi[s * PS:s * PS + D, :] = pi
        pr, pi = _cmul(pr, pi, z1r, z1i)
    z8r_s[...] = pr
    z8i_s[...] = pi
    for _ in range(3):
        pr, pi = pr * pr - pi * pi, 2.0 * pr * pi
    z64r_s[...] = pr
    z64i_s[...] = pi
    pr, pi = pr * pr - pi * pi, 2.0 * pr * pi
    qr, qi = wr, wi
    for a in range(8):
        war[a * PS:a * PS + D, :] = qr
        wai[a * PS:a * PS + D, :] = -qi
        qr, qi = _cmul(qr, qi, pr, pi)
    for _ in range(3):
        pr, pi = pr * pr - pi * pi, 2.0 * pr * pi
    zkr_s[...] = pr
    zki_s[...] = pi

    KU = 4

    cp_x.wait()

    def kgen(gg, _):
        blk = x_ref[pl.ds(pl.multiple_of(gg * 128, 128), 128), :].T.astype(F32)
        xT[gg] = blk
        lo = lax.broadcasted_iota(jnp.int32, (16, 128), 1) < 64

        def row(ref, d):
            return jnp.broadcast_to(ref[pl.ds(d, 1), :], (8, 128))

        for q in range(KU):
            g = gg * KU + q
            outs = []
            for j in range(4):
                lr, li, tr, ti = [], [], [], []
                for d in (g * 8 + 2 * j, g * 8 + 2 * j + 1):
                    a0r = war[pl.ds(d, 8, stride=PS), :]
                    a0i = wai[pl.ds(d, 8, stride=PS), :]
                    zkr, zki = row(zkr_s, d), row(zki_s, d)
                    zhr, zhi = row(z64r_s, d), row(z64i_s, d)
                    a1r = a0r * zkr + a0i * zki
                    a1i = a0i * zkr - a0r * zki
                    lr += [a0r, a1r, a0r * zhr + a0i * zhi, a1r * zhr + a1i * zhi]
                    li += [a0i, a1i, a0i * zhr - a0r * zhi, a1i * zhr - a1r * zhi]
                    er = zbr[pl.ds(d, 8, stride=PS), :]
                    ei = zbi[pl.ds(d, 8, stride=PS), :]
                    z8r, z8i = row(z8r_s, d), row(z8i_s, d)
                    tr.append(er)
                    ti.append(ei)
                    for i in range(7):
                        er, ei = _cmul(er, ei, z8r, z8i)
                        tr.append(er)
                        ti.append(ei)
                lhs = jnp.concatenate([jnp.concatenate(lr, axis=0),
                                       jnp.concatenate(li, axis=0)], axis=1).astype(BF)
                rhs = jnp.concatenate([jnp.concatenate(tr, axis=0),
                                       jnp.concatenate(ti, axis=0)], axis=1).astype(BF)
                o = _mm(lhs, rhs, _NTD)
                ev = jnp.where(lo, o[0:16], o[32:48])
                od = jnp.where(lo, o[16:32], o[48:64])
                outs.append(jnp.where(lo, ev, pltpu.roll(od, 64, 1)))
                outs.append(jnp.where(lo, pltpu.roll(ev, 64, 1), od))
            kt_s[g] = jnp.concatenate(outs, axis=0).astype(BF)
        return _
    lax.fori_loop(0, D // 8 // KU, kgen, None)

    def st1k(gg, _):
        tiles = [kt_s[gg * SU + j] for j in range(SU)]
        res = _mm(s1k_ref[...], jnp.concatenate(tiles, axis=1))
        for j in range(SU):
            sl = pl.ds(pl.multiple_of((gg * SU + j) * 8, 8), 8)
            pln[:, sl, :] = res[:, 128 * j:128 * (j + 1)].reshape(32, 8, 128)
        return _
    lax.fori_loop(0, D // 8 // SU, st1k, None)
    cp_f2.wait()

    inv_n = 1.0 / NFFT
    for k in (0, 16):
        fr_, fi_ = fft_stage2_fwd(k, True)
        kf[k, 0] = fr_ * inv_n
        kf[k, 1] = fi_ * inv_n

    def kf_loop(kk, _):
        for u in range(TU):
            k = 1 + kk * TU + u
            fr_, fi_ = fft_stage2_fwd(k, False)
            kf[k, 0] = fr_ * inv_n
            kf[k, 1] = fi_ * inv_n
        return _
    lax.fori_loop(0, 15 // TU, kf_loop, None)

    cp_w.wait()
    cp_wo.wait()
    r = iota((128, 128), 0)
    c = iota((128, 128), 1)
    bmask = (r % 8) == (c // 16)
    pmat = ((r // 8 == c % 16) & (r % 8 == c // 16)).astype(BF)
    wp2 = wphi_ref[...].reshape(256, 32)
    rx = (iota((128, 256), 0) // 8 == iota((128, 256), 1) % 16).astype(BF)
    sel = (iota((32, D), 0) == iota((32, D), 1) // 16).astype(BF)
    uall = _mm(wp2, sel)
    vall = jnp.where(iota((256, D), 0) // 16 == iota((256, D), 1) % 16, uall, 0.0).astype(BF)
    bdT = _mm(rx, vall)
    for g in range(4):
        bg = jnp.where(bmask, bdT[:, 128 * g:128 * (g + 1)], 0.0).astype(BF)
        wT[128 * g:128 * (g + 1), :] = _mm(bg, wqkv_ref[:, 128 * g:128 * (g + 1)], _NTD).astype(BF)
        wT[512 + 128 * g:512 + 128 * (g + 1), :] = _mm(
            bg, wqkv_ref[:, 512 + 128 * g:512 + 128 * (g + 1)], _NTD).astype(BF)
        wT[1024 + 128 * g:1024 + 128 * (g + 1), :] = _mm(
            pmat, wqkv_ref[:, 1024 + 128 * g:1024 + 128 * (g + 1)], _NTD).astype(BF)
        wog = _mm(pmat, wo_ref[128 * g:128 * (g + 1), :])
        woT[:, 128 * g:128 * (g + 1)] = wog.T.astype(BF)

    def load_chunk(ref, i):
        return jnp.concatenate([ref[i * CT + t] for t in range(CT)], axis=1)

    def store_chunk(ref, i, val):
        for t in range(CT):
            ref[i * CT + t] = val[:, 128 * t:128 * (t + 1)]

    def layer(_l, _c):
        kvacc[...] = jnp.zeros(kvacc.shape, F32)
        zacc[...] = jnp.zeros(zacc.shape, F32)

        def ln_chunk(i):
            store_chunk(xn_s, i, _layernorm_cols(load_chunk(xT, i)).astype(BF))


        def pass1(ii, _):
            for u in range(AU):
                i = ii * AU + u
                ln_chunk(i)
                xn = load_chunk(xn_s, i)
                kvp = _mm(wT[512:1536, :], xn)
                for g in range(4):
                    phi = _dual_softmax(kvp[128 * g:128 * (g + 1)])
                    vg = kvp[512 + 128 * g:512 + 128 * (g + 1)].astype(BF)
                    kvacc[g] += _mm(phi.astype(BF), vg, _NTD)
                    zs = phi[:, 0:128]
                    for t in range(1, CT):
                        zs = zs + phi[:, 128 * t:128 * (t + 1)]
                    zacc[g] += zs
            return _
        lax.fori_loop(0, NT // CT // AU, pass1, None)

        hm = (iota((144, 256), 0) % 8) == (iota((144, 256), 1) % 8)
        for g in range(4):
            zcol = jnp.sum(zacc[g], axis=1, keepdims=True)
            ext = jnp.concatenate([kvacc[g], jnp.broadcast_to(zcol, (256, 128))], axis=1)
            extT = ext.T
            kvT[g] = jnp.where(hm, extT[0:144], 0.0).astype(BF)

        def pass2(ii, _):
            for u in range(AU):
                i = ii * AU + u
                xn = load_chunk(xn_s, i)
                pq = _mm(wT[0:512, :], xn)
                os_ = []
                for g in range(4):
                    phi = _dual_softmax(pq[128 * g:128 * (g + 1)]).astype(BF)
                    nd = _mm(kvT[g], phi)
                    rden = 1.0 / (nd[128:136] + 1e-6)
                    os_.append((nd[0:128].reshape(16, 8, C) * rden[None]).reshape(128, C))
                o = jnp.concatenate(os_, axis=0).astype(BF)
                xnew = load_chunk(xT, i) + _mm(woT[...], o)
                store_chunk(xT, i, xnew)
                store_chunk(uT, i, _layernorm_cols(xnew))
            return _
        lax.fori_loop(0, NT // CT // AU, pass2, None)

        def st1(gg, _):
            tiles = []
            for j in range(SU):
                sl = pl.ds(pl.multiple_of((gg * SU + j) * 8, 8), 8)
                tiles.append(uT[:, sl, :].reshape(128, 128).astype(BF))
            res = _mm(s1_ref[...], jnp.concatenate(tiles, axis=1))
            for j in range(SU):
                sl = pl.ds(pl.multiple_of((gg * SU + j) * 8, 8), 8)
                pln[:, sl, :] = res[:, 128 * j:128 * (j + 1)].reshape(32, 8, 128)
            return _
        lax.fori_loop(0, D // 8 // SU, st1, None)

        for k in (0, 16):
            ur, ui = fft_stage2_fwd(k, True)
            yr, yi = _cmul(ur, ui, kf[k, 0], kf[k, 1])
            pln[k] = (_mm(yr.astype(BF), f2_ref[k, 0], _NTD)
                      + _mm(yi.astype(BF), f2_ref[k, 1], _NTD))

        def st23(kk, _):
            for u in range(TU):
                k = 1 + kk * TU + u
                ur, ui = fft_stage2_fwd(k, False)
                yr, yi = _cmul(ur, ui, kf[k, 0], kf[k, 1])
                q1 = _mm((yr + yi).astype(BF), f2_ref[k, 0], _NTD)
                q2 = _mm(yr.astype(BF), f2_ref[k, 1], _NTD)
                q3 = _mm(yi.astype(BF), f2_ref[k, 2], _NTD)
                pln[k] = q1 + q3
                pln[16 + k] = q1 - q2
            return _
        lax.fori_loop(0, 15 // TU, st23, None)

        def st4(gg, _):
            tiles = []
            for j in range(SU):
                sl = pl.ds(pl.multiple_of((gg * SU + j) * 8, 8), 8)
                tiles.append(pln[:, sl, :].reshape(256, 128).astype(BF))
            res = _mm(s4_ref[...], jnp.concatenate(tiles, axis=1))
            for j in range(SU):
                sl = pl.ds(pl.multiple_of((gg * SU + j) * 8, 8), 8)
                y = res[:, 128 * j:128 * (j + 1)].reshape(16, 8, 128)
                xT[:, sl, :] = xT[:, sl, :] + y + uT[:, sl, :] * dskb[sl, :][None]
            return _
        lax.fori_loop(0, D // 8 // SU, st4, None)
        return _c

    lax.fori_loop(0, 2, layer, None)

    ocps = []
    for ch in range(4):
        for j in range(4):
            i = ch * 4 + j
            o_ref[i * 128:(i + 1) * 128, :] = xT[i].astype(o_ref.dtype).T
        cp = pltpu.make_async_copy(o_ref.at[pl.ds(ch * 512, 512), :], o_hbm.at[pl.ds(ch * 512, 512), :],
                                   osems.at[ch])
        cp.start()
        ocps.append(cp)
    for cp in ocps:
        cp.wait()


def _build(interpret=False):
    def run(A_x, A_wqkv, A_w_phi, A_wo, B_u, B_A_re, B_A_im, B_B_re, B_B_im, B_C_re, B_C_im,
            B_log_dt, B_Dskip):
        del B_u
        x2 = A_x.reshape(S, D)
        wphi, ldt, dsk = jnp.transpose(A_w_phi, (1, 2, 0)), B_log_dt, B_Dskip
        scratch = [
            pltpu.VMEM((S, D), BF),
            pltpu.VMEM((D, 3 * D), BF),
            pltpu.VMEM((D, D), BF),
            pltpu.VMEM((17, 3, 128, 128), BF),
            pltpu.VMEM((S, D), A_x.dtype),
            pltpu.VMEM((64, 128, 128), BF),
            pltpu.SemaphoreType.DMA((4,)),
            pltpu.SemaphoreType.DMA((4,)),
            pltpu.VMEM((NT, D, 128), F32),
            pltpu.VMEM((NT, D, 128), F32),
            pltpu.VMEM((NT, D, 128), BF),
            pltpu.VMEM((32, D, 128), F32),
            pltpu.VMEM((17, 2, D, 128), F32),
            pltpu.VMEM((3 * D, D), BF),
            pltpu.VMEM((D, D), BF),
            pltpu.VMEM((4, 256, 128), F32),
            pltpu.VMEM((4, 256, 128), F32),
            pltpu.VMEM((4, 144, 256), BF),
            pltpu.VMEM((8 * PS, 128), F32),
            pltpu.VMEM((8 * PS, 128), F32),
            pltpu.VMEM((8 * PS, 128), F32),
            pltpu.VMEM((8 * PS, 128), F32),
            pltpu.VMEM((D, 128), F32),
            pltpu.VMEM((D, 128), F32),
            pltpu.VMEM((D, 128), F32),
            pltpu.VMEM((D, 128), F32),
            pltpu.VMEM((D, 128), F32),
            pltpu.VMEM((D, 128), F32),
            pltpu.VMEM((D, 128), F32),
        ]
        any_ = pl.BlockSpec(memory_space=pl.ANY)
        vm = pl.BlockSpec(memory_space=pltpu.VMEM)
        out = pl.pallas_call(
            _kernel,
            out_shape=jax.ShapeDtypeStruct((S, D), A_x.dtype),
            scratch_shapes=scratch,
            in_specs=[any_, any_, vm, any_] + [vm] * 11 + [any_],
            out_specs=any_,
            compiler_params=pltpu.CompilerParams(vmem_limit_bytes=100 * 1024 * 1024),
            interpret=interpret,
        )(x2, A_wqkv, wphi, A_wo, B_A_re, B_A_im, B_B_re, B_B_im, B_C_re, B_C_im, ldt, dsk,
          _S1, _S1K, _S4, _F2)
        return out.reshape(A_x.shape)
    return run


pallas_interleave_layers__linear_kernel_hedgehog__ssm_conv_s4__prompt_kernel = jax.jit(_build(False))
```

```python
import numpy as np
import jax
import jax.numpy as jnp
from jax import lax
import jax.experimental.pallas as pl
import jax.experimental.pallas.tpu as pltpu

S = 2048
D = 512
NT = 16
PS = 513
NFFT = 4096
BF = jnp.bfloat16
F32 = jnp.float32


def _dft_constants():
    n1 = np.arange(16)[None, :]
    k1 = np.arange(17)[:, None]
    ang = -2.0 * np.pi * (n1 * k1) / 32.0
    f1 = np.concatenate([np.cos(ang), np.sin(ang)[1:16]], axis=0)
    eye8 = np.eye(8)
    s1 = np.kron(f1, eye8)
    s1k = np.einsum("pn,ab->panb", f1, eye8)
    s1k = np.transpose(s1k, (0, 1, 3, 2)).reshape(256, 128)
    n1c = np.arange(16)[:, None]
    k1r = np.arange(17)[None, :]
    ang2 = 2.0 * np.pi * (n1c * k1r) / 32.0
    wre = 2.0 * np.cos(ang2)
    wre[:, 0] = 1.0
    wre[:, 16] = np.cos(np.pi * np.arange(16))
    wim = -2.0 * np.sin(ang2)[:, 1:16]
    g4 = np.concatenate([wre, wim], axis=1)
    s4 = np.kron(g4, eye8)
    n2 = np.arange(128)[:, None]
    k2 = np.arange(128)[None, :]
    f2 = np.zeros((17, 3, 128, 128), np.float64)
    for k in range(17):
        a = -2.0 * np.pi * ((n2 * (k + 32 * k2)) % NFFT) / NFFT
        fr, fi = np.cos(a), np.sin(a)
        f2[k, 0] = fr
        if k in (0, 16):
            f2[k, 1] = fi
            f2[k, 2] = fi
        else:
            f2[k, 1] = fr + fi
            f2[k, 2] = fi - fr
    import ml_dtypes
    bf = ml_dtypes.bfloat16
    return (s1.astype(np.float32).astype(bf), s1k.astype(np.float32).astype(bf),
            s4.astype(np.float32).astype(bf), f2.astype(np.float32).astype(bf))


_S1, _S1K, _S4, _F2 = _dft_constants()

_NN = (((1,), (0,)), ((), ()))
_NTD = (((1,), (1,)), ((), ()))


def _mm(a, b, dn=_NN):
    return lax.dot_general(a, b, dn, preferred_element_type=F32)


def _cmul(ar, ai, br, bi):
    return ar * br - ai * bi, ar * bi + ai * br


def _sincos(x):
    kq = jnp.round(x * 0.6366197723675814)
    r = x - kq * 1.5703125
    r = r - kq * 4.837512969970703e-4
    r = r - kq * 7.549790126404332e-8
    r2 = r * r
    sn = r + r * r2 * (-1.6666654611e-1 + r2 * (8.3321608736e-3 + r2 * -1.9515295891e-4))
    cs = 1.0 + r2 * (-0.5 + r2 * (4.166664568298827e-2 + r2 * (-1.388731625493765e-3 + r2 * 2.443315711809948e-5)))
    ki = kq.astype(jnp.int32)
    swap = (ki & 1) == 1
    s_ = jnp.where(swap, cs, sn)
    c_ = jnp.where(swap, sn, cs)
    s_ = jnp.where((ki & 2) == 2, -s_, s_)
    c_ = jnp.where(((ki + 1) & 2) == 2, -c_, c_)
    return s_, c_


def _layernorm_cols(x):
    m = jnp.mean(x, axis=0, keepdims=True)
    xc = x - m
    v = jnp.mean(xc * xc, axis=0, keepdims=True)
    return xc * lax.rsqrt(v + 1e-5)


def _dual_softmax(p):
    c = p.shape[1]
    p3 = p.reshape(16, 8, c)
    mx = jnp.max(p3, axis=0, keepdims=True)
    mn = jnp.min(p3, axis=0, keepdims=True)
    ep = jnp.exp(p3 - mx)
    en = jnp.exp(mn - p3)
    rp = 1.0 / jnp.sum(ep, axis=0, keepdims=True)
    rn = 1.0 / jnp.sum(en, axis=0, keepdims=True)
    return jnp.concatenate([(ep * rp).reshape(128, c), (en * rn).reshape(128, c)], axis=0)


def _kernel(x_hbm, wqkv_hbm, wphi_ref, wo_hbm, are_ref, aim_ref, bre_ref, bim_ref,
            cre_ref, cim_ref, ldt_ref, dsk_ref, s1_ref, s1k_ref, s4_ref, f2_hbm,
            o_hbm,
            x_ref, wqkv_ref, wo_ref, f2_ref, o_ref, kt_s, sems, osems,
            xT, uT, xn_s, pln, kf, wT, woT, kvacc, zacc, kvT, zbr, zbi, war, wai, dskb, z8r_s, z8i_s, zkr_s, zki_s, z64r_s, z64i_s, kend_s):
    SU = 64
    AU = 1
    TU = 15
    CT = 8
    C = 128 * CT

    cp_f2 = pltpu.make_async_copy(f2_hbm, f2_ref, sems.at[0])
    cp_w = pltpu.make_async_copy(wqkv_hbm, wqkv_ref, sems.at[1])
    cp_wo = pltpu.make_async_copy(wo_hbm, wo_ref, sems.at[2])
    cp_x = pltpu.make_async_copy(x_hbm, x_ref, sems.at[3])
    cp_x.start()
    cp_f2.start()
    cp_w.start()
    cp_wo.start()

    def iota(shape, dim):
        return lax.broadcasted_iota(jnp.int32, shape, dim)

    ldt = jnp.broadcast_to(ldt_ref[...].astype(F32).reshape(1, D), (128, D)).T
    dt = jnp.exp(ldt).astype(BF).astype(F32)
    dskb[...] = jnp.broadcast_to(dsk_ref[...].astype(F32).reshape(1, D), (128, D)).T

    def fft_stage2_fwd(k, first):
        ar = pln[k]
        if first:
            arb = ar.astype(BF)
            return _mm(arb, f2_ref[k, 0]), _mm(arb, f2_ref[k, 1])
        ai = pln[16 + k]
        p1 = _mm((ar + ai).astype(BF), f2_ref[k, 0])
        p2 = _mm(ai.astype(BF), f2_ref[k, 1])
        p3 = _mm(ar.astype(BF), f2_ref[k, 2])
        return p1 - p2, p1 + p3

    lam_r = dt * are_ref[...].astype(F32)
    lam_i = dt * aim_ref[...].astype(F32)
    mag = jnp.exp(lam_r)
    sn_, cs_ = _sincos(lam_i)
    z1r = mag * cs_
    z1i = mag * sn_
    dbr = dt * bre_ref[...].astype(F32)
    dbi = dt * bim_ref[...].astype(F32)
    wr, wi = _cmul(cre_ref[...].astype(F32), cim_ref[...].astype(F32), dbr, dbi)
    pr = jnp.ones_like(z1r)
    pi = jnp.zeros_like(z1r)
    for s in range(8):
        zbr[s * PS:s * PS + D, :] = pr
        zbi[s * PS:s * PS + D, :] = pi
        pr, pi = _cmul(pr, pi, z1r, z1i)
    z8r_s[...] = pr
    z8i_s[...] = pi
    for _ in range(3):
        pr, pi = pr * pr - pi * pi, 2.0 * pr * pi
    z64r_s[...] = pr
    z64i_s[...] = pi
    pr, pi = pr * pr - pi * pi, 2.0 * pr * pi
    qr, qi = wr, wi
    for a in range(8):
        war[a * PS:a * PS + D, :] = qr
        wai[a * PS:a * PS + D, :] = -qi
        qr, qi = _cmul(qr, qi, pr, pi)
    for _ in range(3):
        pr, pi = pr * pr - pi * pi, 2.0 * pr * pi
    zkr_s[...] = pr
    zki_s[...] = pi
    pr, pi = pr * pr - pi * pi, 2.0 * pr * pi
    kend_s[...] = jnp.broadcast_to(jnp.sum(wr * pr - wi * pi, axis=1, keepdims=True), (D, 128))

    KU = 4

    cp_x.wait()

    def kgen(gg, _):
        blk = x_ref[pl.ds(pl.multiple_of(gg * 128, 128), 128), :].T.astype(F32)
        xT[gg] = blk
        lo = lax.broadcasted_iota(jnp.int32, (16, 128), 1) < 64

        n1_ = lax.broadcasted_iota(jnp.int32, (16, 128), 0)
        n2_ = lax.broadcasted_iota(jnp.int32, (16, 128), 1)
        sh = jnp.where(n1_ < 2, 0, jnp.where(n1_ < 4, 1, jnp.where(n1_ < 8, 2, 3)))
        half = jnp.where(sh > 0, (1 << sh) // 2 - 1 + ((n2_ >> sh) & 1), 0)
        rq = ((n2_ + half) >> sh) << sh
        wrap = rq == 128
        qidx = rq & 127

        def quantize_l(t, d):
            kend = jnp.broadcast_to(kend_s[pl.ds(d, 1), :], (16, 128))
            nxt = jnp.where(n1_ == 15, kend, pltpu.roll(t, 15, 0))
            nxt0 = jnp.broadcast_to(nxt[:, 0:1], (16, 128))
            return jnp.where(wrap, nxt0, jnp.take_along_axis(t, qidx, axis=1))

        def row(ref, d):
            return jnp.broadcast_to(ref[pl.ds(d, 1), :], (8, 128))

        for q in range(KU):
            g = gg * KU + q
            outs = []
            for j in range(4):
                lr, li, tr, ti = [], [], [], []
                for d in (g * 8 + 2 * j, g * 8 + 2 * j + 1):
                    a0r = war[pl.ds(d, 8, stride=PS), :]
                    a0i = wai[pl.ds(d, 8, stride=PS), :]
                    zkr, zki = row(zkr_s, d), row(zki_s, d)
                    zhr, zhi = row(z64r_s, d), row(z64i_s, d)
                    a1r = a0r * zkr + a0i * zki
                    a1i = a0i * zkr - a0r * zki
                    lr += [a0r, a1r, a0r * zhr + a0i * zhi, a1r * zhr + a1i * zhi]
                    li += [a0i, a1i, a0i * zhr - a0r * zhi, a1i * zhr - a1r * zhi]
                    er = zbr[pl.ds(d, 8, stride=PS), :]
                    ei = zbi[pl.ds(d, 8, stride=PS), :]
                    z8r, z8i = row(z8r_s, d), row(z8i_s, d)
                    tr.append(er)
                    ti.append(ei)
                    for i in range(7):
                        er, ei = _cmul(er, ei, z8r, z8i)
                        tr.append(er)
                        ti.append(ei)
                lhs = jnp.concatenate([jnp.concatenate(lr, axis=0),
                                       jnp.concatenate(li, axis=0)], axis=1).astype(BF)
                rhs = jnp.concatenate([jnp.concatenate(tr, axis=0),
                                       jnp.concatenate(ti, axis=0)], axis=1).astype(BF)
                o = _mm(lhs, rhs, _NTD)
                ev = jnp.where(lo, o[0:16], o[32:48])
                od = jnp.where(lo, o[16:32], o[48:64])
                outs.append(quantize_l(jnp.where(lo, ev, pltpu.roll(od, 64, 1)), g * 8 + 2 * j))
                outs.append(quantize_l(jnp.where(lo, pltpu.roll(ev, 64, 1), od), g * 8 + 2 * j + 1))
            kt_s[g] = jnp.concatenate(outs, axis=0).astype(BF)
        return _
    lax.fori_loop(0, D // 8 // KU, kgen, None)

    def st1k(gg, _):
        tiles = [kt_s[gg * SU + j] for j in range(SU)]
        res = _mm(s1k_ref[...], jnp.concatenate(tiles, axis=1))
        for j in range(SU):
            sl = pl.ds((gg * SU + j) * 8, 8)
            pln[:, sl, :] = res[:, 128 * j:128 * (j + 1)].reshape(32, 8, 128)
        return _
    st1k(0, None)
    cp_f2.wait()

    inv_n = 1.0 / NFFT
    for k in (0, 16):
        fr_, fi_ = fft_stage2_fwd(k, True)
        kf[k, 0] = fr_ * inv_n
        kf[k, 1] = fi_ * inv_n

    def kf_loop(kk, _):
        for u in range(TU):
            k = 1 + kk * TU + u
            fr_, fi_ = fft_stage2_fwd(k, False)
            kf[k, 0] = fr_ * inv_n
            kf[k, 1] = fi_ * inv_n
        return _
    kf_loop(0, None)

    cp_w.wait()
    cp_wo.wait()
    r = iota((128, 128), 0)
    c = iota((128, 128), 1)
    bmask = (r % 8) == (c // 16)
    pmat = ((r // 8 == c % 16) & (r % 8 == c // 16)).astype(BF)
    wp2 = wphi_ref[...].reshape(256, 32)
    rx = (iota((128, 256), 0) // 8 == iota((128, 256), 1) % 16).astype(BF)
    sel = (iota((32, D), 0) == iota((32, D), 1) // 16).astype(BF)
    uall = _mm(wp2, sel)
    vall = jnp.where(iota((256, D), 0) // 16 == iota((256, D), 1) % 16, uall, 0.0).astype(BF)
    bdT = _mm(rx, vall)
    for g in range(4):
        bg = jnp.where(bmask, bdT[:, 128 * g:128 * (g + 1)], 0.0).astype(BF)
        wT[128 * g:128 * (g + 1), :] = _mm(bg, wqkv_ref[:, 128 * g:128 * (g + 1)], _NTD).astype(BF)
        wT[512 + 128 * g:512 + 128 * (g + 1), :] = _mm(
            bg, wqkv_ref[:, 512 + 128 * g:512 + 128 * (g + 1)], _NTD).astype(BF)
        wT[1024 + 128 * g:1024 + 128 * (g + 1), :] = _mm(
            pmat, wqkv_ref[:, 1024 + 128 * g:1024 + 128 * (g + 1)], _NTD).astype(BF)
        wog = _mm(pmat, wo_ref[128 * g:128 * (g + 1), :])
        woT[:, 128 * g:128 * (g + 1)] = wog.T.astype(BF)

    def load_chunk(ref, i):
        return jnp.concatenate([ref[i * CT + t] for t in range(CT)], axis=1)

    def store_chunk(ref, i, val):
        for t in range(CT):
            ref[i * CT + t] = val[:, 128 * t:128 * (t + 1)]

    def layer(_l, _c):
        kvacc[...] = jnp.zeros(kvacc.shape, F32)
        zacc[...] = jnp.zeros(zacc.shape, F32)

        def ln_chunk(i):
            store_chunk(xn_s, i, _layernorm_cols(load_chunk(xT, i)).astype(BF))


        def pass1(ii, _):
            for u in range(AU):
                i = ii * AU + u
                ln_chunk(i)
                xn = load_chunk(xn_s, i)
                kvp = _mm(wT[512:1536, :], xn)
                for g in range(4):
                    phi = _dual_softmax(kvp[128 * g:128 * (g + 1)])
                    vg = kvp[512 + 128 * g:512 + 128 * (g + 1)].astype(BF)
                    kvacc[g] += _mm(phi.astype(BF), vg, _NTD)
                    zs = phi[:, 0:128]
                    for t in range(1, CT):
                        zs = zs + phi[:, 128 * t:128 * (t + 1)]
                    zacc[g] += zs
            return _
        lax.fori_loop(0, NT // CT // AU, pass1, None)

        hm = (iota((144, 256), 0) % 8) == (iota((144, 256), 1) % 8)
        for g in range(4):
            zcol = jnp.sum(zacc[g], axis=1, keepdims=True)
            ext = jnp.concatenate([kvacc[g], jnp.broadcast_to(zcol, (256, 128))], axis=1)
            extT = ext.T
            kvT[g] = jnp.where(hm, extT[0:144], 0.0).astype(BF)

        def pass2(ii, _):
            for u in range(AU):
                i = ii * AU + u
                xn = load_chunk(xn_s, i)
                pq = _mm(wT[0:512, :], xn)
                os_ = []
                for g in range(4):
                    phi = _dual_softmax(pq[128 * g:128 * (g + 1)]).astype(BF)
                    nd = _mm(kvT[g], phi)
                    rden = 1.0 / (nd[128:136] + 1e-6)
                    os_.append((nd[0:128].reshape(16, 8, C) * rden[None]).reshape(128, C))
                o = jnp.concatenate(os_, axis=0).astype(BF)
                xnew = load_chunk(xT, i) + _mm(woT[...], o)
                store_chunk(xT, i, xnew)
                store_chunk(uT, i, _layernorm_cols(xnew))
            return _
        lax.fori_loop(0, NT // CT // AU, pass2, None)

        def st1(gg, _):
            tiles = []
            for j in range(SU):
                sl = pl.ds((gg * SU + j) * 8, 8)
                tiles.append(uT[:, sl, :].reshape(128, 128).astype(BF))
            res = _mm(s1_ref[...], jnp.concatenate(tiles, axis=1))
            for j in range(SU):
                sl = pl.ds((gg * SU + j) * 8, 8)
                pln[:, sl, :] = res[:, 128 * j:128 * (j + 1)].reshape(32, 8, 128)
            return _
        st1(0, None)

        for k in (0, 16):
            ur, ui = fft_stage2_fwd(k, True)
            yr, yi = _cmul(ur, ui, kf[k, 0], kf[k, 1])
            pln[k] = (_mm(yr.astype(BF), f2_ref[k, 0], _NTD)
                      + _mm(yi.astype(BF), f2_ref[k, 1], _NTD))

        def st23(kk, _):
            for u in range(TU):
                k = 1 + kk * TU + u
                ur, ui = fft_stage2_fwd(k, False)
                yr, yi = _cmul(ur, ui, kf[k, 0], kf[k, 1])
                q1 = _mm((yr + yi).astype(BF), f2_ref[k, 0], _NTD)
                q2 = _mm(yr.astype(BF), f2_ref[k, 1], _NTD)
                q3 = _mm(yi.astype(BF), f2_ref[k, 2], _NTD)
                pln[k] = q1 + q3
                pln[16 + k] = q1 - q2
            return _
        st23(0, None)

        def st4(gg, _):
            tiles = []
            for j in range(SU):
                sl = pl.ds((gg * SU + j) * 8, 8)
                tiles.append(pln[:, sl, :].reshape(256, 128).astype(BF))
            res = _mm(s4_ref[...], jnp.concatenate(tiles, axis=1))
            for j in range(SU):
                sl = pl.ds((gg * SU + j) * 8, 8)
                y = res[:, 128 * j:128 * (j + 1)].reshape(16, 8, 128)
                xT[:, sl, :] = xT[:, sl, :] + y + uT[:, sl, :] * dskb[sl, :][None]
            return _
        st4(0, None)
        return _c

    lax.fori_loop(0, 2, layer, None)

    ocps = []
    for ch in range(4):
        for j in range(4):
            i = ch * 4 + j
            o_ref[i * 128:(i + 1) * 128, :] = xT[i].astype(o_ref.dtype).T
        cp = pltpu.make_async_copy(o_ref.at[pl.ds(ch * 512, 512), :], o_hbm.at[pl.ds(ch * 512, 512), :],
                                   osems.at[ch])
        cp.start()
        ocps.append(cp)
    for cp in ocps:
        cp.wait()


def _build(interpret=False):
    def run(A_x, A_wqkv, A_w_phi, A_wo, B_u, B_A_re, B_A_im, B_B_re, B_B_im, B_C_re, B_C_im,
            B_log_dt, B_Dskip):
        del B_u
        x2 = A_x.reshape(S, D)
        wphi, ldt, dsk = jnp.transpose(A_w_phi, (1, 2, 0)), B_log_dt, B_Dskip
        scratch = [
            pltpu.VMEM((S, D), BF),
            pltpu.VMEM((D, 3 * D), BF),
            pltpu.VMEM((D, D), BF),
            pltpu.VMEM((17, 3, 128, 128), BF),
            pltpu.VMEM((S, D), A_x.dtype),
            pltpu.VMEM((64, 128, 128), BF),
            pltpu.SemaphoreType.DMA((4,)),
            pltpu.SemaphoreType.DMA((4,)),
            pltpu.VMEM((NT, D, 128), F32),
            pltpu.VMEM((NT, D, 128), F32),
            pltpu.VMEM((NT, D, 128), BF),
            pltpu.VMEM((32, D, 128), F32),
            pltpu.VMEM((17, 2, D, 128), F32),
            pltpu.VMEM((3 * D, D), BF),
            pltpu.VMEM((D, D), BF),
            pltpu.VMEM((4, 256, 128), F32),
            pltpu.VMEM((4, 256, 128), F32),
            pltpu.VMEM((4, 144, 256), BF),
            pltpu.VMEM((8 * PS, 128), F32),
            pltpu.VMEM((8 * PS, 128), F32),
            pltpu.VMEM((8 * PS, 128), F32),
            pltpu.VMEM((8 * PS, 128), F32),
            pltpu.VMEM((D, 128), F32),
            pltpu.VMEM((D, 128), F32),
            pltpu.VMEM((D, 128), F32),
            pltpu.VMEM((D, 128), F32),
            pltpu.VMEM((D, 128), F32),
            pltpu.VMEM((D, 128), F32),
            pltpu.VMEM((D, 128), F32),
            pltpu.VMEM((D, 128), F32),
        ]
        any_ = pl.BlockSpec(memory_space=pl.ANY)
        vm = pl.BlockSpec(memory_space=pltpu.VMEM)
        out = pl.pallas_call(
            _kernel,
            out_shape=jax.ShapeDtypeStruct((S, D), A_x.dtype),
            scratch_shapes=scratch,
            in_specs=[any_, any_, vm, any_] + [vm] * 11 + [any_],
            out_specs=any_,
            compiler_params=pltpu.CompilerParams(vmem_limit_bytes=100 * 1024 * 1024),
            interpret=interpret,
        )(x2, A_wqkv, wphi, A_wo, B_A_re, B_A_im, B_B_re, B_B_im, B_C_re, B_C_im, ldt, dsk,
          _S1, _S1K, _S4, _F2)
        return out.reshape(A_x.shape)
    return run


pallas_interleave_layers__linear_kernel_hedgehog__ssm_conv_s4__prompt_kernel = jax.jit(_build(False))
```
